```python
import jax
import jax.numpy as jnp

def _softmax(x, axis=-1):
    return jax.nn.softmax(x, axis=axis)

def _gelu(x):
    return jax.nn.gelu(x, approximate=True)

def _silu(x):
    return jax.nn.silu(x)

def _sigmoid(x):
    return jax.nn.sigmoid(x)

def _layernorm(x, axis=-1, eps=1e-05):
    m = jnp.mean(x, axis=axis, keepdims=True)
    v = jnp.var(x, axis=axis, keepdims=True)
    return (x - m) / jnp.sqrt(v + eps)

def _scatter_add(tgt, idx, src, axis=0):
    return tgt.at[idx].add(src)

def _segment_sum(src, seg, n):
    return jax.ops.segment_sum(src, seg, n)

class _Rng:

    def __init__(self, key):
        self._k = key

    def _next(self):
        self._k, sub = jax.random.split(self._k)
        return sub

    def normal(self, shape):
        return jax.random.normal(self._next(), shape, dtype=jnp.bfloat16)

    def randint(self, lo, hi, shape):
        return jax.random.randint(self._next(), shape, lo, hi, dtype=jnp.int32)

    def uniform(self, shape, lo=0.0, hi=1.0):
        return jax.random.uniform(self._next(), shape, jnp.bfloat16, lo, hi)

    def permutation(self, n):
        return jax.random.permutation(self._next(), n)
kernel_name = 'standalone__conformer_conv_module__speech'

def setup_inputs():
    _rng = _Rng(jax.random.key(int.from_bytes(__import__("os").urandom(4), "little")))
    _w = lambda a: (lambda t: t.astype(jnp.bfloat16) if jnp.issubdtype(t.dtype, jnp.floating) else t)(jnp.asarray(a))
    B, T, D, K = (2, 16000, 256, 31)
    return {'x': _w((lambda *s: _rng.normal(s) * 0.05)(B, T, D)), 'w_pw1': _w((lambda *s: _rng.normal(s) * 0.05)(D, 2 * D)), 'dw': _w((lambda *s: _rng.normal(s) * 0.05)(K, D)), 'w_pw2': _w((lambda *s: _rng.normal(s) * 0.05)(D, D))}

def reference(x, w_pw1, dw, w_pw2):
    B, T, D = x.shape
    K = dw.shape[0]
    h = x @ w_pw1
    a, b = (h[..., :D].copy(), h[..., D:].copy())
    h = a * _sigmoid(b)
    pad = K // 2
    hp = jnp.pad(h, ((0, 0), (pad, pad), (0, 0)))
    out = jnp.zeros_like(h)
    for i in range(K):
        out = out + hp[:, i:i + T, :] * dw[i][None, None, :]
    return _silu(out) @ w_pw2
```

```python
import functools
import jax
import jax.numpy as jnp
import jax.experimental.pallas as pl
import jax.experimental.pallas.tpu as pltpu

TT = 800
R = 160


def _kernel(xp_ref, x_ref, xn_ref, w1_ref, dw_ref, w2_ref, o_ref, h_ref, *, nt):
    j = pl.program_id(1)
    D = w2_ref.shape[0]
    K = dw_ref.shape[0]
    w1 = (w1_ref[...].astype(jnp.float32) * 0.5).astype(jnp.bfloat16)
    dw = dw_ref[...].astype(jnp.float32) * 0.5
    w2 = w2_ref[...]

    def glu(xv):
        ab = jnp.dot(xv, w1, preferred_element_type=jnp.float32)
        a, b = ab[:, :D], ab[:, D:]
        return a * jnp.tanh(b) + a

    def put(r0, h):
        n = h.shape[0]
        for c in range(D // 128):
            h_ref[c, pl.ds(r0, n), :] = h[:, c * 128:(c + 1) * 128]

    put(0, jnp.where(j > 0, glu(xp_ref[...]), 0.0))
    put(16 + TT, jnp.where(j < nt - 1, glu(xn_ref[...]), 0.0))
    for r in range(0, TT, R):
        put(16 + r, glu(x_ref[r:r + R, :]))
    for r in range(0, TT, R):
        cols = []
        for c in range(D // 128):
            acc = None
            for k in range(K):
                t = h_ref[c, pl.ds(r + 1 + k, R), :] * dw[k:k + 1, c * 128:(c + 1) * 128]
                acc = t if acc is None else acc + t
            cols.append((acc * jnp.tanh(acc) + acc).astype(jnp.bfloat16))
        s = jnp.concatenate(cols, axis=1)
        o_ref[r:r + R, :] = jnp.dot(s, w2, preferred_element_type=jnp.float32).astype(o_ref.dtype)


@jax.jit
def pallas_standalone__conformer_conv_module__speech_kernel(x, w_pw1, dw, w_pw2):
    B, T, D = x.shape
    nt = T // TT
    hb = TT // 16
    return pl.pallas_call(
        functools.partial(_kernel, nt=nt),
        grid=(B, nt),
        in_specs=[
            pl.BlockSpec((None, 16, D), lambda b, j: (b, jnp.maximum(j * hb - 1, 0), 0)),
            pl.BlockSpec((None, TT, D), lambda b, j: (b, j, 0)),
            pl.BlockSpec((None, 16, D), lambda b, j: (b, jnp.minimum((j + 1) * hb, T // 16 - 1), 0)),
            pl.BlockSpec(w_pw1.shape, lambda b, j: (0, 0)),
            pl.BlockSpec(dw.shape, lambda b, j: (0, 0)),
            pl.BlockSpec(w_pw2.shape, lambda b, j: (0, 0)),
        ],
        out_specs=pl.BlockSpec((None, TT, D), lambda b, j: (b, j, 0)),
        out_shape=jax.ShapeDtypeStruct(x.shape, x.dtype),
        scratch_shapes=[pltpu.VMEM((D // 128, TT + 32, 128), jnp.float32)],
        compiler_params=pltpu.CompilerParams(dimension_semantics=("parallel", "parallel")),
    )(x, x, x, w_pw1, dw, w_pw2)
```

```python
import functools
import jax
import jax.numpy as jnp
import jax.experimental.pallas as pl
import jax.experimental.pallas.tpu as pltpu

TT = 3200
R = 320
G = 16

f32 = jnp.float32
bf16 = jnp.bfloat16


def _split(w):
    e, o = w[0::2], w[1::2]
    return [e, [a if b is None else a + b for a, b in zip(e, o)], o]


def _kernel(xp_ref, x_ref, xn_ref, w1_ref, dw_ref, w2_ref, o_ref,
            h_ref, u_ref, s_ref, w1s_ref, w2s_ref, wt_ref, *, nt):
    j = pl.program_id(1)
    D = w2_ref.shape[0]
    K = dw_ref.shape[0]
    NC = D // 128

    @pl.when((pl.program_id(0) == 0) & (j == 0))
    def _():
        w1s_ref[...] = pltpu.bitcast((w1_ref[...].astype(f32) * 0.5).astype(bf16), jnp.int32)
        w2s_ref[...] = pltpu.bitcast(w2_ref[...], jnp.int32)
        dw = dw_ref[...].astype(f32) * 0.5
        taps = [dw[k:k + 1] for k in range(K)] + [None]
        for a, f in enumerate(_split(taps)):
            for b, g in enumerate(_split(f)):
                for k, t in enumerate(g):
                    if t is not None:
                        wt_ref[(a * 3 + b) * 8 + k] = jnp.broadcast_to(t, (8, D))
        h_ref[:, TT + 32:, :] = jnp.zeros((NC, 8, 128), f32)

    def glu(xv):
        ab = jnp.dot(xv, pltpu.bitcast(w1s_ref[...], bf16), preferred_element_type=f32)
        a, b = ab[:, :D], ab[:, D:]
        return a * jnp.tanh(b) + a

    def put(r0, h):
        for c in range(NC):
            h_ref[c, pl.ds(r0, h.shape[0]), :] = h[:, c * 128:(c + 1) * 128]

    def streams(m0, n):
        for c in range(NC):
            p = [h_ref[c, pl.ds(4 * m0 + 1 + i, n, stride=4), :] for i in range(7)]
            l1 = [(p[0] - p[1], p[2] - p[3], p[4] - p[5]),
                  (p[1], p[3], p[5]),
                  (p[2] - p[1], p[4] - p[3], p[6] - p[5])]
            for a, (u0, u1, u2) in enumerate(l1):
                u_ref[c, a * 3 + 0, pl.ds(m0, n), :] = u0 - u1
                u_ref[c, a * 3 + 1, pl.ds(m0, n), :] = u1
                u_ref[c, a * 3 + 2, pl.ds(m0, n), :] = u2 - u1

    def conv(m0, n):
        nv = n // 8
        for c in range(NC):
            def conv_c(c=c):
                def corr(acc, s):
                    for k in range(7 if s == 8 else 8):
                        w = wt_ref[s * 8 + k, :, c * 128:(c + 1) * 128]
                        t = [u_ref[c, s, pl.ds(m0 + k + 8 * v, 8), :] * w for v in range(nv)]
                        acc = t if acc is None else [p + q for p, q in zip(acc, t)]
                    return acc
                mm = corr(None, 4)
                me, mo = corr(mm, 3), corr(mm, 5)
                for a, ph in ((0, 0), (2, 1)):
                    t = corr(None, a * 3 + 1)
                    for q, base in ((0, me), (1, mo)):
                        ys = corr([p + r for p, r in zip(t, base)], a * 3 + 2 * q)
                        for v, y in enumerate(ys):
                            s_ref[c, pl.ds(4 * (m0 + 8 * v) + ph + 2 * q, 8, stride=4), :] = y * jnp.tanh(y) + y
            yield conv_c

    def mm2(r):
        s = jnp.concatenate([s_ref[c, r:r + R, :] for c in range(NC)], axis=1).astype(bf16)
        o_ref[r:r + R, :] = jnp.dot(s, pltpu.bitcast(w2s_ref[...], bf16), preferred_element_type=f32).astype(o_ref.dtype)

    n = TT // R
    Q = R // 4
    put(0, jnp.where(j > 0, glu(xp_ref[...]), 0.0))
    for i in range(n + 3):
        cv = [f for g in range(0, Q, G) for f in conv((i - 2) * Q + g, G)] if 2 <= i <= n + 1 else []
        if i < n:
            put(16 + i * R, glu(x_ref[i * R:(i + 1) * R, :]))
        elif i == n:
            put(16 + TT, jnp.where(j < nt - 1, glu(xn_ref[...]), 0.0))
        for f in cv[:len(cv) // 2]:
            f()
        if 3 <= i:
            mm2((i - 3) * R)
        if i <= n:
            streams(i * Q, Q if i < n else 8)
        for f in cv[len(cv) // 2:]:
            f()


@jax.jit
def pallas_standalone__conformer_conv_module__speech_kernel(x, w_pw1, dw, w_pw2):
    B, T, D = x.shape
    nt = T // TT
    hb = TT // 16
    NC = D // 128
    return pl.pallas_call(
        functools.partial(_kernel, nt=nt),
        grid=(B, nt),
        in_specs=[
            pl.BlockSpec((None, 16, D), lambda b, j: (b, jnp.maximum(j * hb - 1, 0), 0)),
            pl.BlockSpec((None, TT, D), lambda b, j: (b, j, 0)),
            pl.BlockSpec((None, 16, D), lambda b, j: (b, jnp.minimum((j + 1) * hb, T // 16 - 1), 0)),
            pl.BlockSpec(w_pw1.shape, lambda b, j: (0, 0)),
            pl.BlockSpec(dw.shape, lambda b, j: (0, 0)),
            pl.BlockSpec(w_pw2.shape, lambda b, j: (0, 0)),
        ],
        out_specs=pl.BlockSpec((None, TT, D), lambda b, j: (b, j, 0)),
        out_shape=jax.ShapeDtypeStruct(x.shape, x.dtype),
        scratch_shapes=[
            pltpu.VMEM((NC, TT + 40, 128), f32),
            pltpu.VMEM((NC, 9, TT // 4 + 8, 128), f32),
            pltpu.VMEM((NC, TT, 128), f32),
            pltpu.VMEM((D // 2, 2 * D), jnp.int32),
            pltpu.VMEM((D // 2, D), jnp.int32),
            pltpu.VMEM((72, 8, D), f32),
        ],
        compiler_params=pltpu.CompilerParams(dimension_semantics=("arbitrary", "arbitrary"), vmem_limit_bytes=64 * 2**20, flags={"XLA_TPU_EVENLY_DISTRIBUTE_CRITICAL_NODES": True}),
    )(x, x, x, w_pw1, dw, w_pw2)
```

```python
import functools
import jax
import jax.numpy as jnp
import jax.experimental.pallas as pl
import jax.experimental.pallas.tpu as pltpu

TT = 1600
R = 320
G = 16

LV = 2
P = 2 ** LV
NS = 3 ** LV
KS = 32 // P

f32 = jnp.float32
bf16 = jnp.bfloat16


def _split(w):
    e, o = w[0::2], w[1::2]
    return [e, [a if b is None else a + b for a, b in zip(e, o)], o]


def _kernel(xp_ref, x_ref, xn_ref, w1_ref, dw_ref, w2_ref, o_ref,
            h_ref, u_ref, s_ref, w1s_ref, w2s_ref, wt_ref, *, nt):
    j = pl.program_id(1)
    D = w2_ref.shape[0]
    K = dw_ref.shape[0]
    NC = D // 128

    @pl.when((pl.program_id(0) == 0) & (j == 0))
    def _():
        w1s_ref[...] = pltpu.bitcast((w1_ref[...].astype(f32) * 0.5).astype(bf16), jnp.int32)
        w2s_ref[...] = pltpu.bitcast(w2_ref[...], jnp.int32)
        dw = dw_ref[...].astype(f32) * 0.5
        taps = [dw[k:k + 1] for k in range(K)] + [None]
        fs = [taps]
        for _ in range(LV):
            fs = [g for f in fs for g in _split(f)]
        for a, g in enumerate(fs):
            for k, t in enumerate(g):
                if t is not None:
                    wt_ref[a * KS + k] = jnp.broadcast_to(t, (8, D))
        h_ref[:, TT + 32:, :] = jnp.zeros((NC, 10 * P - 32, 128), f32)

    def glu(xv):
        ab = jnp.dot(xv, pltpu.bitcast(w1s_ref[...], bf16), preferred_element_type=f32)
        a, b = ab[:, :D], ab[:, D:]
        return a * jnp.tanh(b) + a

    def put(r0, h):
        for c in range(NC):
            h_ref[c, pl.ds(r0, h.shape[0]), :] = h[:, c * 128:(c + 1) * 128]

    def streams(m0, n):
        for c in range(NC):
            us = [[h_ref[c, pl.ds(P * m0 + 1 + i, n, stride=P), :] for i in range(2 * P - 1)]]
            for _ in range(LV):
                us = [g for u in us for g in (
                    [a - b for a, b in zip(u[0::2], u[1::2])], u[1::2],
                    [a - b for a, b in zip(u[2::2], u[1::2])])]
            for a, u in enumerate(us):
                u_ref[c, a, pl.ds(m0, n), :] = u[0]

    def conv(m0, n):
        for c in range(NC):
            def conv_c(c=c):
                def node(lv, s):
                    if lv == LV:
                        acc = None
                        for k in range(KS - 1 if s == NS - 1 else KS):
                            w = wt_ref[s * KS + k, :, c * 128:(c + 1) * 128]
                            t = u_ref[c, s, pl.ds(m0 + k, n), :].reshape(n // 8, 8, 128) * w[None]
                            acc = t if acc is None else acc + t
                        return [acc]
                    e, m, o = (node(lv + 1, 3 * s + b) for b in range(3))
                    return [y for ev, mv, ov in zip(e, m, o) for y in (ev + mv, ov + mv)]
                for ph, y in enumerate(node(0, 0)):
                    s_ref[c, pl.ds(P * m0 + ph, n, stride=P), :] = (y * jnp.tanh(y) + y).reshape(n, 128)
            yield conv_c

    def mm2(r):
        s = jnp.concatenate([s_ref[c, r:r + R, :] for c in range(NC)], axis=1).astype(bf16)
        o_ref[r:r + R, :] = jnp.dot(s, pltpu.bitcast(w2s_ref[...], bf16), preferred_element_type=f32).astype(o_ref.dtype)

    n = TT // R
    Q = R // P
    put(0, jnp.where(j > 0, glu(xp_ref[...]), 0.0))
    for i in range(n + 3):
        cv = [f for g in range(0, Q, G) for f in conv((i - 2) * Q + g, G)] if 2 <= i <= n + 1 else []
        if i < n:
            put(16 + i * R, glu(x_ref[i * R:(i + 1) * R, :]))
        elif i == n:
            put(16 + TT, jnp.where(j < nt - 1, glu(xn_ref[...]), 0.0))
        for f in cv[:len(cv) // 2]:
            f()
        if 3 <= i:
            mm2((i - 3) * R)
        if i <= n:
            streams(i * Q, Q if i < n else 8)
        for f in cv[len(cv) // 2:]:
            f()


@jax.jit
def pallas_standalone__conformer_conv_module__speech_kernel(x, w_pw1, dw, w_pw2):
    B, T, D = x.shape
    nt = T // TT
    hb = TT // 16
    NC = D // 128
    return pl.pallas_call(
        functools.partial(_kernel, nt=nt),
        grid=(B, nt),
        in_specs=[
            pl.BlockSpec((None, 16, D), lambda b, j: (b, jnp.maximum(j * hb - 1, 0), 0)),
            pl.BlockSpec((None, TT, D), lambda b, j: (b, j, 0)),
            pl.BlockSpec((None, 16, D), lambda b, j: (b, jnp.minimum((j + 1) * hb, T // 16 - 1), 0)),
            pl.BlockSpec(w_pw1.shape, lambda b, j: (0, 0)),
            pl.BlockSpec(dw.shape, lambda b, j: (0, 0)),
            pl.BlockSpec(w_pw2.shape, lambda b, j: (0, 0)),
        ],
        out_specs=pl.BlockSpec((None, TT, D), lambda b, j: (b, j, 0)),
        out_shape=jax.ShapeDtypeStruct(x.shape, x.dtype),
        scratch_shapes=[
            pltpu.VMEM((NC, TT + 10 * P, 128), f32),
            pltpu.VMEM((NC, NS, TT // P + 8, 128), f32),
            pltpu.VMEM((NC, TT, 128), f32),
            pltpu.VMEM((D // 2, 2 * D), jnp.int32),
            pltpu.VMEM((D // 2, D), jnp.int32),
            pltpu.VMEM((NS * KS, 8, D), f32),
        ],
        compiler_params=pltpu.CompilerParams(dimension_semantics=("arbitrary", "arbitrary"), vmem_limit_bytes=64 * 2**20),
    )(x, x, x, w_pw1, dw, w_pw2)
```

```python
import functools
import jax
import jax.numpy as jnp
import jax.experimental.pallas as pl
import jax.experimental.pallas.tpu as pltpu

TT = 1600
R = 320
BAR = 0
G = 16

LV = 2
P = 2 ** LV
NS = 3 ** LV
KS = 32 // P

f32 = jnp.float32
bf16 = jnp.bfloat16


def _split(w):
    e, o = w[0::2], w[1::2]
    return [e, [a if b is None else a + b for a, b in zip(e, o)], o]


def _kernel(xp_ref, x_ref, xn_ref, w1_ref, dw_ref, w2_ref, o_ref,
            h_ref, u_ref, m_ref, s_ref, w1s_ref, w2s_ref, wt_ref, *, nt):
    j = pl.program_id(1)
    D = w2_ref.shape[0]
    K = dw_ref.shape[0]
    NC = D // 128

    @pl.when((pl.program_id(0) == 0) & (j == 0))
    def _():
        w1 = w1_ref[...].astype(f32) * 0.5
        for c in range(NC):
            wc = jnp.concatenate([w1[:, c * 128:(c + 1) * 128], w1[:, D + c * 128:D + (c + 1) * 128]], axis=1)
            w1s_ref[c] = pltpu.bitcast(wc.astype(bf16), jnp.int32)
        w2s_ref[...] = pltpu.bitcast(w2_ref[...], jnp.int32)
        dw = dw_ref[...].astype(f32) * 0.5
        taps = [dw[k:k + 1] for k in range(K)] + [None]
        fs = [taps]
        for _ in range(LV):
            fs = [g for f in fs for g in _split(f)]
        for a, g in enumerate(fs):
            for k, t in enumerate(g):
                if t is not None:
                    wt_ref[a * KS + k] = jnp.broadcast_to(t, (8, D))
        h_ref[:, TT + 32:, :] = jnp.zeros((NC, 10 * P - 32, 128), f32)

    def glu(c, i):
        lo, hi = i * R, (i + 1) * R
        xs = [x_ref[lo:hi, :]]
        if i == 0:
            xs.insert(0, jnp.where(j > 0, xp_ref[...], jnp.zeros((), bf16)))
        if i == n - 1:
            xs.append(jnp.where(j < nt - 1, xn_ref[...], jnp.zeros((), bf16)))
        ab = jnp.dot(jnp.concatenate(xs, axis=0), pltpu.bitcast(w1s_ref[c], bf16), preferred_element_type=f32)
        a, b = ab[:, :128], ab[:, 128:]
        h_ref[c, pl.ds(0 if i == 0 else lo + 16, a.shape[0]), :] = a * jnp.tanh(b) + a

    def streams(c, i):
        m0, nq = i * Q, Q + (8 if i == n - 1 else 0)
        us = [[h_ref[c, pl.ds(P * m0 + 1 + k, nq, stride=P), :] for k in range(2 * P - 1)]]
        for _ in range(LV):
            us = [g for u in us for g in (
                [a - b for a, b in zip(u[0::2], u[1::2])], u[1::2],
                [a - b for a, b in zip(u[2::2], u[1::2])])]
        for a, u in enumerate(us):
            u_ref[c, a, pl.ds(m0, nq), :] = u[0]

    def conv(c, i, a):
        m0 = i * Q
        def leaf(s):
            acc = None
            for k in range(KS - 1 if s == NS - 1 else KS):
                w = wt_ref[s * KS + k, :, c * 128:(c + 1) * 128]
                t = u_ref[c, s, pl.ds(m0 + k, Q), :].reshape(Q // 8, 8, 128) * w[None]
                acc = t if acc is None else acc + t
            return acc.reshape(Q, 128)
        m = leaf(3 * a + 1)
        for q in (0, 1):
            y = leaf(3 * a + 2 * q) + m
            if a == 1:
                m_ref[c, q, pl.ds(m0, Q), :] = y
            else:
                y = y + m_ref[c, q, pl.ds(m0, Q), :]
                s_ref[c, pl.ds(P * m0 + a // 2 + 2 * q, Q, stride=P), :] = y * jnp.tanh(y) + y

    def mm2(r, nr):
        s = jnp.concatenate([s_ref[c, r:r + nr, :] for c in range(NC)], axis=1).astype(bf16)
        o_ref[r:r + nr, :] = jnp.dot(s, pltpu.bitcast(w2s_ref[...], bf16), preferred_element_type=f32).astype(o_ref.dtype)

    n = TT // R
    Q = R // P
    ok = lambda i: 0 <= i < n
    for i in range(n + 4):
        for p, a in enumerate((1, 0, 2)):
            def blk():
                if p < 2:
                    if ok(i):
                        glu(p, i)
                elif ok(i - 4):
                    mm2((i - 4) * R, R)
                for c in range(NC):
                    if ok(i - 3):
                        conv(c, i - 3, a)
                if p == 2:
                    for c in range(NC):
                        if ok(i - 1):
                            streams(c, i - 1)
            if BAR:
                pl.when(j >= 0)(blk)
            else:
                blk()


@jax.jit
def pallas_standalone__conformer_conv_module__speech_kernel(x, w_pw1, dw, w_pw2):
    B, T, D = x.shape
    nt = T // TT
    hb = TT // 16
    NC = D // 128
    return pl.pallas_call(
        functools.partial(_kernel, nt=nt),
        grid=(B, nt),
        in_specs=[
            pl.BlockSpec((None, 16, D), lambda b, j: (b, jnp.maximum(j * hb - 1, 0), 0)),
            pl.BlockSpec((None, TT, D), lambda b, j: (b, j, 0)),
            pl.BlockSpec((None, 16, D), lambda b, j: (b, jnp.minimum((j + 1) * hb, T // 16 - 1), 0)),
            pl.BlockSpec(w_pw1.shape, lambda b, j: (0, 0)),
            pl.BlockSpec(dw.shape, lambda b, j: (0, 0)),
            pl.BlockSpec(w_pw2.shape, lambda b, j: (0, 0)),
        ],
        out_specs=pl.BlockSpec((None, TT, D), lambda b, j: (b, j, 0)),
        out_shape=jax.ShapeDtypeStruct(x.shape, x.dtype),
        scratch_shapes=[
            pltpu.VMEM((NC, TT + 10 * P, 128), f32),
            pltpu.VMEM((NC, NS, TT // P + 8, 128), f32),
            pltpu.VMEM((NC, 2, TT // P, 128), f32),
            pltpu.VMEM((NC, TT, 128), f32),
            pltpu.VMEM((NC, D // 2, 256), jnp.int32),
            pltpu.VMEM((D // 2, D), jnp.int32),
            pltpu.VMEM((NS * KS, 8, D), f32),
        ],
        compiler_params=pltpu.CompilerParams(dimension_semantics=("arbitrary", "arbitrary"), vmem_limit_bytes=64 * 2**20),
    )(x, x, x, w_pw1, dw, w_pw2)
```

```python
import functools
import jax
import jax.numpy as jnp
import jax.experimental.pallas as pl
import jax.experimental.pallas.tpu as pltpu

TT = 1600
R = 320

LV = 2
P = 2 ** LV
NS = 3 ** LV
KS = 32 // P

f32 = jnp.float32
bf16 = jnp.bfloat16


def _split(w):
    e, o = w[0::2], w[1::2]
    return [e, [a if b is None else a + b for a, b in zip(e, o)], o]


def _kernel(xp_ref, x_ref, xn_ref, w1_ref, dw_ref, w2_ref, o_ref,
            h_ref, u_ref, m_ref, s_ref, w1s_ref, w2s_ref, wt_ref, *, nt):
    j = pl.program_id(1)
    D = w2_ref.shape[0]
    K = dw_ref.shape[0]
    NC = D // 128

    @pl.when((pl.program_id(0) == 0) & (j == 0))
    def _():
        w1 = w1_ref[...].astype(f32) * 0.5
        for c in range(NC):
            wc = jnp.concatenate([w1[:, c * 128:(c + 1) * 128], w1[:, D + c * 128:D + (c + 1) * 128]], axis=1)
            w1s_ref[c] = pltpu.bitcast(wc.astype(bf16), jnp.int32)
        w2s_ref[...] = pltpu.bitcast(w2_ref[...], jnp.int32)
        dw = dw_ref[...].astype(f32) * 0.5
        taps = [dw[k:k + 1] for k in range(K)] + [None]
        fs = [taps]
        for _ in range(LV):
            fs = [g for f in fs for g in _split(f)]
        for a, g in enumerate(fs):
            for k, t in enumerate(g):
                if t is not None:
                    wt_ref[a * KS + k] = jnp.broadcast_to(t, (8, D))
        h_ref[:, TT + 32:, :] = jnp.zeros((NC, 10 * P - 32, 128), f32)

    def glu(c, i):
        lo, hi = i * R, (i + 1) * R
        xs = [x_ref[lo:hi, :]]
        if i == 0:
            xs.insert(0, jnp.where(j > 0, xp_ref[...], jnp.zeros((), bf16)))
        if i == n - 1:
            xs.append(jnp.where(j < nt - 1, xn_ref[...], jnp.zeros((), bf16)))
        ab = jnp.dot(jnp.concatenate(xs, axis=0), pltpu.bitcast(w1s_ref[c], bf16), preferred_element_type=f32)
        a, b = ab[:, :128], ab[:, 128:]
        h_ref[c, pl.ds(0 if i == 0 else lo + 16, a.shape[0]), :] = a * jnp.tanh(b) + a

    def streams(c, i):
        m0, nq = i * Q, Q + (8 if i == n - 1 else 0)
        us = [[h_ref[c, pl.ds(P * m0 + 1 + k, nq, stride=P), :] for k in range(2 * P - 1)]]
        for _ in range(LV):
            us = [g for u in us for g in (
                [a - b for a, b in zip(u[0::2], u[1::2])], u[1::2],
                [a - b for a, b in zip(u[2::2], u[1::2])])]
        for a, u in enumerate(us):
            u_ref[c, a, pl.ds(m0, nq), :] = u[0]

    def conv(c, i, a):
        m0 = i * Q
        def leaf(s):
            acc = None
            for k in range(KS - 1 if s == NS - 1 else KS):
                w = wt_ref[s * KS + k, :, c * 128:(c + 1) * 128]
                t = u_ref[c, s, pl.ds(m0 + k, Q), :].reshape(Q // 8, 8, 128) * w[None]
                acc = t if acc is None else acc + t
            return acc.reshape(Q, 128)
        m = leaf(3 * a + 1)
        for q in (0, 1):
            y = leaf(3 * a + 2 * q) + m
            if a == 1:
                m_ref[c, q, pl.ds(m0, Q), :] = y
            else:
                y = y + m_ref[c, q, pl.ds(m0, Q), :]
                s_ref[c, pl.ds(P * m0 + a // 2 + 2 * q, Q, stride=P), :] = y * jnp.tanh(y) + y

    def mm2(r, nr):
        s = jnp.concatenate([s_ref[c, r:r + nr, :] for c in range(NC)], axis=1).astype(bf16)
        o_ref[r:r + nr, :] = jnp.dot(s, pltpu.bitcast(w2s_ref[...], bf16), preferred_element_type=f32).astype(o_ref.dtype)

    n = TT // R
    Q = R // P
    ok = lambda i: 0 <= i < n
    for i in range(n + 4):
        for p, a in enumerate((1, 0, 2)):
            def blk():
                if p < 2:
                    if ok(i):
                        glu(p, i)
                elif ok(i - 3):
                    mm2((i - 3) * R, R)
                for c in range(NC):
                    if ok(i - 2):
                        conv(c, i - 2, a)
                if p == 2:
                    for c in range(NC):
                        if ok(i):
                            streams(c, i)
            blk()


@jax.jit
def pallas_standalone__conformer_conv_module__speech_kernel(x, w_pw1, dw, w_pw2):
    B, T, D = x.shape
    nt = T // TT
    hb = TT // 16
    NC = D // 128
    return pl.pallas_call(
        functools.partial(_kernel, nt=nt),
        grid=(B, nt),
        in_specs=[
            pl.BlockSpec((None, 16, D), lambda b, j: (b, jnp.maximum(j * hb - 1, 0), 0)),
            pl.BlockSpec((None, TT, D), lambda b, j: (b, j, 0)),
            pl.BlockSpec((None, 16, D), lambda b, j: (b, jnp.minimum((j + 1) * hb, T // 16 - 1), 0)),
            pl.BlockSpec(w_pw1.shape, lambda b, j: (0, 0)),
            pl.BlockSpec(dw.shape, lambda b, j: (0, 0)),
            pl.BlockSpec(w_pw2.shape, lambda b, j: (0, 0)),
        ],
        out_specs=pl.BlockSpec((None, TT, D), lambda b, j: (b, j, 0)),
        out_shape=jax.ShapeDtypeStruct(x.shape, x.dtype),
        scratch_shapes=[
            pltpu.VMEM((NC, TT + 10 * P, 128), f32),
            pltpu.VMEM((NC, NS, TT // P + 8, 128), f32),
            pltpu.VMEM((NC, 2, TT // P, 128), f32),
            pltpu.VMEM((NC, TT, 128), f32),
            pltpu.VMEM((NC, D // 2, 256), jnp.int32),
            pltpu.VMEM((D // 2, D), jnp.int32),
            pltpu.VMEM((NS * KS, 8, D), f32),
        ],
        compiler_params=pltpu.CompilerParams(dimension_semantics=("arbitrary", "arbitrary"), vmem_limit_bytes=64 * 2**20),
    )(x, x, x, w_pw1, dw, w_pw2)
```
